```python
import jax
import jax.numpy as jnp

def _softmax(x, axis=-1):
    return jax.nn.softmax(x, axis=axis)

def _gelu(x):
    return jax.nn.gelu(x, approximate=True)

def _silu(x):
    return jax.nn.silu(x)

def _sigmoid(x):
    return jax.nn.sigmoid(x)

def _layernorm(x, axis=-1, eps=1e-05):
    m = jnp.mean(x, axis=axis, keepdims=True)
    v = jnp.var(x, axis=axis, keepdims=True)
    return (x - m) / jnp.sqrt(v + eps)

def _scatter_add(tgt, idx, src, axis=0):
    return tgt.at[idx].add(src)

def _segment_sum(src, seg, n):
    return jax.ops.segment_sum(src, seg, n)

class _Rng:

    def __init__(self, key):
        self._k = key

    def _next(self):
        self._k, sub = jax.random.split(self._k)
        return sub

    def normal(self, shape):
        return jax.random.normal(self._next(), shape, dtype=jnp.bfloat16)

    def randint(self, lo, hi, shape):
        return jax.random.randint(self._next(), shape, lo, hi, dtype=jnp.int32)

    def uniform(self, shape, lo=0.0, hi=1.0):
        return jax.random.uniform(self._next(), shape, jnp.bfloat16, lo, hi)

    def permutation(self, n):
        return jax.random.permutation(self._next(), n)
kernel_name = 'adaLN_cond__ssm_conv_h3__glu_gated_swiglu__prompt'

def setup_inputs():
    _rng = _Rng(jax.random.key(int.from_bytes(__import__("os").urandom(4), "little")))
    _w = lambda a: (lambda t: t.astype(jnp.bfloat16) if jnp.issubdtype(t.dtype, jnp.floating) else t)(jnp.asarray(a))

    def _A_setup():
        B, S, D = (1, 2048, 640)
        ks = 4
        return {'q': _w((lambda *s: _rng.normal(s) * 0.05)(B, S, D)), 'k': _w((lambda *s: _rng.normal(s) * 0.05)(B, S, D)), 'v': _w((lambda *s: _rng.normal(s) * 0.05)(B, S, D)), 'shift_k': _w((lambda *s: _rng.normal(s) * 0.05)(D, ks) * 0.5), 'ssm_k': _w((lambda *s: _rng.normal(s) * 0.05)(D, S) * (1.0 / S ** 0.5)), 'ssm_D': _w((lambda *s: _rng.normal(s) * 0.05)(D))}
    _A_in = _A_setup()

    def _B_setup():
        B, S, D, F = (1, 2048, 640, 1536)
        return {'x': _w((lambda *s: _rng.normal(s) * 0.05)(B, S, D)), 'w1': _w((lambda *s: _rng.normal(s) * 0.05)(D, F) * (2.0 / D) ** 0.5), 'w3': _w((lambda *s: _rng.normal(s) * 0.05)(D, F) * (2.0 / D) ** 0.5), 'w2': _w((lambda *s: _rng.normal(s) * 0.05)(F, D) * (2.0 / F) ** 0.5)}
    _B_in = _B_setup()
    return {'A_q': _A_in['q'], 'A_k': _A_in['k'], 'A_v': _A_in['v'], 'A_shift_k': _A_in['shift_k'], 'A_ssm_k': _A_in['ssm_k'], 'A_ssm_D': _A_in['ssm_D'], 'B_x': _B_in['x'], 'B_w1': _B_in['w1'], 'B_w3': _B_in['w3'], 'B_w2': _B_in['w2'], 'c': _w((lambda *s: _rng.normal(s) * 0.05)(1, 640)), 'w_mod': _w((lambda *s: _rng.normal(s) * 0.05)(640, 6 * 640) * 640 ** (-0.5))}

def reference(A_q, A_k, A_v, A_shift_k, A_ssm_k, A_ssm_D, B_x, B_w1, B_w3, B_w2, c, w_mod):

    def _A_ref(q, k, v, shift_k, ssm_k, ssm_D):
        B, S, D = q.shape
        ks = shift_k.shape[-1]
        k_pad = jnp.pad(k, ((0, 0), (ks - 1, 0), (0, 0)))
        k_shift = jnp.zeros_like(k)
        for t in range(ks):
            k_shift = k_shift + k_pad[:, t:t + S, :] * shift_k[:, ks - 1 - t][None, None, :]
        kv = k_shift * v
        L = 2 * S
        kv_pad = jnp.pad(kv, ((0, 0), (0, S), (0, 0)))
        kf_pad = jnp.pad(ssm_k, ((0, 0), (0, S)))
        kv_f = (lambda x, axes=(-2, -1): jnp.fft.rfft2(x.astype(jnp.float32), axes=axes))(kv_pad[:, None, :, :], axes=(1, 2))
        kf_f = (lambda x, axes=(-2, -1): jnp.fft.rfft2(x.astype(jnp.float32), axes=axes))(kf_pad[:, None, :], axes=(1, 2))
        kf_f = (lambda x, *d: x.transpose(*d))(kf_f, 1, 2, 0)
        y_f = kv_f * kf_f[None, :, :, :]
        y = (lambda x, s, axes=(-2, -1): jnp.fft.irfft2(x, s=s, axes=axes).astype(jnp.bfloat16))(y_f, (1, L), axes=(1, 2))[:, 0, :S, :]
        y = y + kv * ssm_D[None, None, :]
        return q * y

    def _B_ref(x, w1, w3, w2):
        gate = jnp.einsum('bsd,df->bsf', x, w1)
        up = jnp.einsum('bsd,df->bsf', x, w3)
        h = _silu(gate) * up
        out = jnp.einsum('bsf,fd->bsd', h, w2)
        return out
    x = A_q
    mod = (_silu(c) @ w_mod).reshape(c.shape[0], 6, 1, -1)
    sa, ca, ga, sb, cb, gb = (mod[:, 0].copy(), mod[:, 1].copy(), mod[:, 2].copy(), mod[:, 3].copy(), mod[:, 4].copy(), mod[:, 5].copy())
    h = _layernorm(x, axis=-1) * (1 + ca) + sa
    x = x + ga * _A_ref(h, A_k, A_v, A_shift_k, A_ssm_k, A_ssm_D)
    h = _layernorm(x, axis=-1) * (1 + cb) + sb
    x = x + gb * _B_ref(h, B_w1, B_w3, B_w2)
    return x
```

```python
import functools
import numpy as np
import jax
import jax.numpy as jnp
from jax import lax
import jax.experimental.pallas as pl
import jax.experimental.pallas.tpu as pltpu

S, D, FF = 2048, 640, 1536
L = 128
NB = S // L
NL = D // 128
NG = L // 8
EPS = 1e-5
TM = 256
FC = 256
NT = S // TM
CH = 256
KR = 32
LNR = 16
A5 = range(5)
def _region(j, mac):
    return ((j,), (("fu", j - 1), ("fw", j - 1)) + ((("mac", j - 2), ("inv", j - 2)) if mac else ()) + (("gate", j),))


PRO_PAIRS = 4
MID_MACS = ()
MID_INVS = ()
MERGE9 = True
LN1_CHAINS = 8
LN2_SPLIT = 128
SPLIT_LAST = True
LATE_MACS = {(2, 6): ((4, A5, 3), (5, A5, 3)), (4, 6): ((6, A5, 3), (7, A5, 3))}
LATE_INVS = {(3, 0): (4, 5), (5, 0): (6, 7)}
O_WAITS = {3: 0, 5: 1}
RETILE = True
CONV_ONLY = False
SCOPES = False


def _dft_mats():
    ks = np.concatenate([np.arange(0, L, 2), np.arange(1, L, 2)])
    th = 2 * np.pi * (ks + 0.5) / (2 * L)
    j = np.arange(L)
    ang = (th[:, None] * j[None, :]).reshape(L // 8, 1, 8, L)
    Fm = np.concatenate([np.cos(ang), -np.sin(ang)], 1).reshape(2 * L, L)
    Gm = Fm.T / L
    Hm = np.concatenate([-np.sin(ang) - np.cos(ang), np.cos(ang) - np.sin(ang)], 1).reshape(2 * L, L)
    return (np.concatenate([Fm, Hm], 0).astype(jnp.bfloat16), np.ascontiguousarray(Gm).astype(jnp.bfloat16))


def _norm(x):
    m = jnp.sum(x, axis=-1, keepdims=True) * (1.0 / D)
    xc = x - m
    v = jnp.sum(xc * xc, axis=-1, keepdims=True) * (1.0 / D)
    return xc * lax.rsqrt(v + EPS)


def _interleave(main, side):
    n, m, done = len(main), len(side), 0
    for i, f in enumerate(main):
        f()
        upto = (i + 1) * m // n
        while done < upto:
            side[done]()
            done += 1


def _kernel(q_hbm, k_hbm, v_hbm, s_hbm, w1_hbm, w3_hbm, w2_hbm, wm_hbm, sh_hbm, dd_hbm, c_hbm, f_hbm, g_hbm,
            out_hbm,
            q_v, k_v, v_v, s_v, w1_v, w3_v, w2_v, wm_v, sh_v, dd_v, cc_v, f_v, g_v, one_v,
            f2_v, g2_v, s2_v, w1b_v, w3b_v, w2b_v, kv_v, u_v, w_v, c_v, y_v, z_v, h_v, n_v, act0_v, act1_v, out_v, mod_v,
            sems):
    f32, bf16 = jnp.float32, jnp.bfloat16
    n_sem = [0]

    def cp(src, dst):
        n_sem[0] += 1
        return pltpu.make_async_copy(src, dst, sems.at[n_sem[0] - 1])

    import contextlib
    n_scope = [0]

    def wait(cs):
        n_scope[0] += 1
        with (jax.named_scope("wait%02d" % n_scope[0]) if SCOPES else contextlib.nullcontext()):
            for c in cs:
                c.wait()

    def rows(j, n):
        return pl.ds(j * n, n)

    small = [cp(a, b) for i, (a, b) in enumerate(
        [(sh_hbm, sh_v), (f_hbm.at[0:16], one_v), (f_hbm, f_v), (dd_hbm, dd_v), (g_hbm, g_v), (c_hbm, cc_v)])]
    NCH = S // CH
    kvs = [[cp(k_hbm.at[rows(j, CH)], k_v.at[rows(j, CH)]),
            cp(v_hbm.at[rows(j, CH)], v_v.at[rows(j, CH)]),
            cp(s_hbm.at[:, rows(j, CH)], s_v.at[:, rows(j, CH)])] for j in range(NCH)]
    wm_order = (2, 1, 0, 4, 3, 5)
    wm = {j: cp(wm_hbm.at[:, rows(j, D)], wm_v.at[:, rows(j, D)]) for j in range(6)}
    qc = [cp(q_hbm.at[rows(t, TM)], q_v.at[rows(t, TM)]) for t in range(NT)]
    NF = FF // FC
    w13 = [[cp(w1_hbm.at[:, rows(j, FC)], w1_v.at[:, rows(j, FC)]),
            cp(w3_hbm.at[:, rows(j, FC)], w3_v.at[:, rows(j, FC)])] for j in range(NF)]
    w2c = cp(w2_hbm, w2_v)
    oc = [[cp(out_v.at[rows(t, TM)], out_hbm.at[rows(t, TM)])] for t in range(NT - 1)]
    oc.append([cp(out_v.at[rows(i, TM // 2)], out_hbm.at[rows(i, TM // 2)]) for i in (2 * NT - 2, 2 * NT - 1)])

    need = [small[:2] + kvs[0][:2], kvs[0][2:] + small[2:] + kvs[1][:2]]
    need += [kvs[j - 1][2:] + kvs[j][:2] for j in range(2, NCH)] + [kvs[NCH - 1][2:]]
    queue = [c for cs in need for c in cs]
    queue += [wm[2], wm[1], wm[0], qc[0], wm[4], wm[3]] + w13[0] + [qc[1]]
    queue += [c for j in range(1, NF) for c in w13[j]] + [qc[2], wm[5], w2c] + qc[3:]
    issued = [0]

    def issue(n):
        for c in queue[issued[0]:issued[0] + n]:
            c.start()
        issued[0] = min(len(queue), issued[0] + n)

    issue(len(queue))

    def gate(r0, key):
        sh = sh_v[...].astype(f32)
        kb = after(k_v[pl.ds(r0, KR), :], chain.get(key)).astype(f32)
        prev = jnp.zeros((8, D), f32) if r0 == 0 else k_v[pl.ds(r0 - 16, 16), :].astype(f32)[8:]
        kk = jnp.concatenate([prev, kb], axis=0)
        ks = kb * sh[0:1]
        for j in range(1, 4):
            ks = ks + pltpu.roll(kk, j, 0)[8:] * sh[j:j + 1]
        kv = (ks * v_v[pl.ds(r0, KR), :].astype(f32)).astype(bf16)
        kv_v[pl.ds(r0, KR), :] = kv
        link(key, bits(kv))

    def fwd_signal(b):
        u = jnp.dot(f2_v[:2 * L], kv_v[rows(b, L), :], preferred_element_type=f32).reshape(NG, 2, 8, D)
        u_v[b] = jnp.stack([u[:, 0] + u[:, 1], u[:, 0], u[:, 1]], axis=1).reshape(3 * L, D)

    def fwd_filter(b):
        w = lax.dot_general(f2_v[2 * L:], s2_v[:, rows(b, L)], (((1,), (1,)), ((), ())), preferred_element_type=f32)
        w = w.reshape(NG, 2, 8, D)
        if b == 0:
            dd = dd_v[...].astype(f32).reshape(1, 1, D)
            cq, cr = w[:, 0] - dd, w[:, 1] + dd
            w = jnp.stack([cq, cr], axis=1)
        else:
            p = w_v[(b - 1) % 2].reshape(NG, 2, 8, D)
            H = NG // 2
            cq = jnp.concatenate([w[:H, 0] + p[:H, 1], w[H:, 0] - p[H:, 1]], axis=0)
            cr = jnp.concatenate([w[:H, 1] - p[:H, 0], w[H:, 1] + p[H:, 0]], axis=0)
        c_v[b] = jnp.stack([cr - cq, cq, cr], axis=1).reshape(3 * L, D)
        if b + 1 < NB:
            w_v[b % 2] = w.reshape(2 * L, D)

    def always():
        return bits(one_v[...]) != jnp.uint32(0xFFFFFFFF)

    def bits(x):
        return pltpu.bitcast(x, jnp.uint32)

    def fold(x, n):
        parts = [x[r:r + 8, c:c + 128] for r in range(0, x.shape[0], 8) for c in range(0, x.shape[1], 128)]
        outs = [functools.reduce(jnp.bitwise_or, parts[i::n]) for i in range(n)]
        return outs[0] if n == 1 else jnp.concatenate(outs, axis=1)

    def after(x, dep):
        if dep is None:
            return x
        xi = bits(x)
        reps = (xi.shape[0] // 8, xi.shape[1] // 128)
        if dep.shape != xi.shape:
            dep = jnp.tile(fold(dep, 1), reps)
        return pltpu.bitcast(jnp.where(jnp.tile(always(), reps), xi, dep), x.dtype)

    chain = {}

    def link(key, dep):
        dep = fold(dep, 1)
        chain[key] = dep

    def mac(outs, l, g, parts):
        ls = pl.ds(l * 128, 128)
        acc = {}
        for part in parts:
            for m in range(max(outs) + 1):
                for i in part:
                    rs = pl.ds(g * 24 + i * 8, 8)
                    c = c_v[m, rs, ls]
                    if m == 0:
                        c = after(c, chain.get(0))
                    for a in outs:
                        if m <= a:
                            t = c * u_v[a - m, rs, ls]
                            acc[a, i] = t if m == 0 else acc[a, i] + t
            if part is not parts[-1]:
                link(0, jnp.concatenate([bits(acc[a, i]) for a in outs for i in part], axis=1))
        ys = []
        for a in outs:
            k0 = 0.5 * acc[a, 0]
            y = jnp.concatenate([k0 - acc[a, 2], k0 + acc[a, 1]], axis=0).astype(bf16)
            y_v[pl.ds(a * 2 * L + g * 16, 16), ls] = y
            ys.append(bits(y))
        link(0, jnp.concatenate(ys, axis=1))

    def inv(b):
        z_v[rows(b, L), :] = jnp.dot(g2_v[...], y_v[rows(b, 2 * L), :], preferred_element_type=f32)

    def mod(j):
        cc = cc_v[...].astype(f32)
        sc = jnp.broadcast_to(cc * jax.nn.sigmoid(cc), (16, D)).astype(bf16)
        mod_v[j] = jnp.dot(sc, wm_v[:, rows(j, D)], preferred_element_type=f32)[:8]

    def ln(r0, key, n=LNR):
        rs = pl.ds(r0, n)
        sa, ca, ga, sb, cb = [jnp.tile(mod_v[j], (n // 8, 1)) for j in range(5)]
        x = after(q_v[rs, :], chain.get(key)).astype(f32)
        x1 = x + ga * ((_norm(x) * (1 + ca) + sa) * z_v[rs, :])
        z_v[rs, :] = x1
        h = (_norm(x1) * (1 + cb) + sb).astype(bf16)
        h_v[rs, :] = h
        if key:
            link(key, bits(h))

    def ln_first_a(r0):
        rs = pl.ds(r0, LNR)
        sa, ca, ga = [jnp.tile(mod_v[j], (LNR // 8, 1)) for j in range(3)]
        x = q_v[rs, :].astype(f32)
        x1 = x + ga * ((_norm(x) * (1 + ca) + sa) * z_v[rs, :])
        z_v[rs, :] = x1
        n_v[rs, :] = _norm(x1)

    def ln_first_b(r0):
        rs = pl.ds(r0, LNR)
        sb, cb = [jnp.tile(mod_v[j], (LNR // 8, 1)) for j in (3, 4)]
        h_v[rs, :] = (n_v[rs, :] * (1 + cb) + sb).astype(bf16)

    def ln_tile(t):
        for i in range(TM // LNR):
            ln(t * TM + i * LNR, "ln")

    def up(t, j):
        h = h_v[rows(t, TM), :]
        if t == 0 or not RETILE:
            w1, w3 = w1_v[:, rows(j, FC)], w3_v[:, rows(j, FC)]
            if RETILE:
                w1b_v[:, rows(j, FC)] = w1
                w3b_v[:, rows(j, FC)] = w3
        else:
            w1, w3 = w1b_v[:, rows(j, FC)], w3b_v[:, rows(j, FC)]
        g = 0.5 * jnp.dot(h, w1, preferred_element_type=f32)
        u = jnp.dot(h, w3, preferred_element_type=f32)
        (act0_v, act1_v)[t % 2][:, rows(j, FC)] = ((g * jnp.tanh(g) + g) * u).astype(bf16)

    def down(t):
        if t == 0 or not RETILE:
            w2 = w2_v[...]
            if RETILE:
                w2b_v[...] = w2
        else:
            w2 = w2b_v[...]
        n = TM // len(oc[t])
        gb = jnp.tile(mod_v[5], (n // 8, 1))
        for i, c in enumerate(oc[t]):
            o = jnp.dot((act0_v, act1_v)[t % 2][rows(i, n), :], w2, preferred_element_type=f32)
            rs = pl.ds(t * TM + i * n, n)
            out_v[rs, :] = (z_v[rs, :] + gb * o).astype(bf16)
            c.start()

    def run(fs):
        for f in fs:
            f()

    def invs(p):
        inv(2 * p)
        inv(2 * p + 1)

    def macs(p, lanes=range(NL), pace=0):
        parts = {0: ((0, 1, 2),), 1: ((0, 1, 2),), 2: ((0, 1), (2,)), 3: ((0,), (1,), (2,))}[pace]
        for l in lanes:
            for g in range(NG):
                if pace in (0, 3):
                    mac((2 * p, 2 * p + 1), l, g, parts)
                else:
                    mac((2 * p + 1,), l, g, parts)
                    mac((2 * p,), l, g, parts)

    plan = [((0,), (("gate", 0),))] + [_region(j, 2 <= j < PRO_PAIRS + 2) for j in range(1, NCH)]
    for chunks, tasks in plan:
        wait([c for j in chunks for c in need[j]])
        if 1 in chunks:
            f2_v[...] = f_v[...]
            g2_v[...] = g_v[...]
        chain.clear()
        for task in tasks:
            if task[0] == "gate":
                for r0 in range(task[1] * CH, (task[1] + 1) * CH, KR):
                    gate(r0, 0)
            elif task[0] == "fw":
                s2_v[:, rows(task[1], CH)] = s_v[:, rows(task[1], CH)]
                fwd_filter(2 * task[1])
                fwd_filter(2 * task[1] + 1)
            elif task[0] == "fu":
                fwd_signal(2 * task[1])
                fwd_signal(2 * task[1] + 1)
            elif task[0] == "inv":
                invs(task[1])
            else:
                macs(*task[1:])
    wait((need[NCH][0], wm[2], wm[1], wm[0], qc[0]) + ((wm[4], wm[3]) if MERGE9 else ()))
    chain.clear()
    for j in (2, 1, 0):
        mod(j)
    s2_v[:, rows(NCH - 1, CH)] = s_v[:, rows(NCH - 1, CH)]
    for b in (NB - 2, NB - 1):
        fwd_signal(b)
        fwd_filter(b)
    for r0 in range(0, TM, LNR):
        ln_first_a(r0)
    for task in MID_MACS:
        macs(*task)
    if not MERGE9:
        wait((wm[4], wm[3]))
    for p in MID_INVS:
        invs(p)
    for j in (4, 3):
        mod(j)
    for r0 in range(0, TM, LNR):
        ln_first_b(r0)
    def at(*pos):
        for p in LATE_INVS.get(pos, ()):
            invs(p)
        if pos in LATE_MACS:
            chain.pop(0, None)
            for task in LATE_MACS[pos]:
                macs(*task)

    wait(w13[0] + w13[1] + [qc[1]])
    chain.clear()
    for i, r0 in enumerate(range(0, TM, LNR)):
        ln(TM + r0, "ln%d" % (i % LN1_CHAINS))
    up(0, 0)
    up(0, 1)
    up(1, 0)
    wait(w13[2])
    up(1, 1)
    up(0, 2)
    up(1, 2)
    wait(w13[3] + w13[4] + w13[5] + [qc[2]])
    chain.clear()
    for r0 in range(0, LN2_SPLIT, LNR):
        ln(2 * TM + r0, "ln")
    for j in range(3, NF):
        up(0, j)
        up(1, j)
    wait([wm[5], w2c] + qc[3:])
    mod(5)
    chain.clear()
    for r0 in range(LN2_SPLIT, TM, LNR):
        ln(2 * TM + r0, "ln")
    down(0)
    down(1)
    for t in range(2, NT):
        if t in O_WAITS:
            wait(oc[O_WAITS[t]])
            chain.clear()
        for j in range(NF):
            at(t, j)
            if j == 0 and t + 1 < NT:
                ln_tile(t + 1)
            up(t, j)
        at(t, NF)
        down(t)
    wait([c for i, cs in enumerate(oc) if i not in O_WAITS.values() for c in cs])


def pallas_adaLN_cond__ssm_conv_h3__glu_gated_swiglu__prompt_kernel(
        A_q, A_k, A_v, A_shift_k, A_ssm_k, A_ssm_D, B_x, B_w1, B_w3, B_w2, c, w_mod):
    Fm, Gm = _dft_mats()
    f32, bf16 = jnp.float32, jnp.bfloat16
    anyspec = pl.BlockSpec(memory_space=pl.ANY)
    V = pltpu.VMEM
    dma = pltpu.SemaphoreType.DMA
    out = pl.pallas_call(
        _kernel,
        in_specs=[anyspec] * 13,
        out_specs=anyspec,
        out_shape=jax.ShapeDtypeStruct((S, D), bf16),
        scratch_shapes=[
            V((S, D), bf16), V((S, D), bf16), V((S, D), bf16), V((D, S), bf16),
            V((D, FF), bf16), V((D, FF), bf16), V((FF, D), bf16), V((D, 6 * D), bf16),
            V((4, D), bf16), V((D,), bf16), V((1, D), bf16), V((4 * L, L), bf16), V((L, 2 * L), bf16), V((16, L), bf16),
            V((4 * L, L), bf16), V((L, 2 * L), bf16), V((D, S), bf16), V((D, FF), bf16), V((D, FF), bf16), V((FF, D), bf16),
            V((S, D), bf16), V((NB, 3 * L, D), f32), V((2, 2 * L, D), f32), V((NB, 3 * L, D), f32), V((NB * 2 * L, D), bf16),
            V((S, D), f32), V((S, D), bf16), V((TM, D), f32), V((TM, FF), bf16), V((TM, FF), bf16), V((S, D), bf16), V((6, 8, D), f32),
            dma((7 + 3 * S // CH + 6 + 2 * NT + 2 * FF // FC + 1,)),
        ],
        compiler_params=pltpu.CompilerParams(vmem_limit_bytes=110 * 1024 * 1024),
    )(A_q.reshape(S, D), A_k.reshape(S, D), A_v.reshape(S, D), A_ssm_k, B_w1, B_w3, B_w2, w_mod,
      A_shift_k.T, A_ssm_D, c, Fm, Gm)
    return out.reshape(1, S, D)
```

```python
import functools
import numpy as np
import jax
import jax.numpy as jnp
from jax import lax
import jax.experimental.pallas as pl
import jax.experimental.pallas.tpu as pltpu

S, D, FF = 2048, 640, 1536
EPS = 1e-5
L = 128
NB = S // L
NG = L // 8
NL = D // 128
CH = 2 * L
NCH = S // CH
TM = 256
NT = S // TM
FC = 256
NF = FF // FC
KR = 32
LNR = 16
ALL = range(NL)

PROLOGUE = (
    (("gate", 0),),
    (("fu", 0), ("fw", 0), ("gate", 1)),
    (("fu", 1), ("fw", 1), ("mac", 0, ALL), ("inv", 0, ALL), ("gate", 2)),
    (("fu", 2), ("fw", 2), ("mac", 1, ALL), ("inv", 1, ALL), ("gate", 3)),
    (("fu", 3), ("fw", 3), ("mac", 2, (0, 1, 2, 3)), ("inv", 2, (0, 1, 2, 3)), ("gate", 4)),
    (("fu", 4), ("fw", 4), ("mac", 2, (4,)), ("mac", 3, (0, 1)), ("inv", 2, (4,)), ("inv", 3, (0, 1)), ("gate", 5)),
    (("fu", 5), ("fw", 5), ("mac", 3, (2, 3, 4)), ("inv", 3, (2, 3, 4)), ("gate", 6), ("gate", 7)),
    (("fu", 6), ("fw", 6), ("fu", 7), ("fw", 7)),
)
LATE = {
    (2, NF): (("mac", 4, ALL, True), ("mac", 5, (0, 1), True)),
    (3, 0): (("inv", 4, ALL),),
    (3, NF): (("mac", 5, (2, 3, 4), True), ("mac", 6, (0, 1), True)),
    (4, 0): (("inv", 5, ALL),),
    (4, NF): (("mac", 6, (2, 3, 4), True), ("mac", 7, (0,), True)),
    (5, 0): (("inv", 6, ALL),),
    (5, NF): (("mac", 7, (1, 2, 3, 4), True),),
    (6, 0): (("inv", 7, ALL),),
}
LN1_CUTS = (0, 96, 192, 256)
LAST_PARTS = ((0, 192), (192, 64))
N_COPIES = 6 + 3 * NCH + 6 + NT + 2 * NF + 1 + (NT - 1) + len(LAST_PARTS)


def _dft_mats():
    ks = np.concatenate([np.arange(0, L, 2), np.arange(1, L, 2)])
    th = 2 * np.pi * (ks + 0.5) / (2 * L)
    j = np.arange(L)
    ang = (th[:, None] * j[None, :]).reshape(L // 8, 1, 8, L)
    Fm = np.concatenate([np.cos(ang), -np.sin(ang)], 1).reshape(2 * L, L)
    Gm = Fm.T / L
    Hm = np.concatenate([-np.sin(ang) - np.cos(ang), np.cos(ang) - np.sin(ang)], 1).reshape(2 * L, L)
    return (np.concatenate([Fm, Hm], 0).astype(jnp.bfloat16), np.ascontiguousarray(Gm).astype(jnp.bfloat16))


def _norm(x):
    m = jnp.sum(x, axis=-1, keepdims=True) * (1.0 / D)
    xc = x - m
    v = jnp.sum(xc * xc, axis=-1, keepdims=True) * (1.0 / D)
    return xc * lax.rsqrt(v + EPS)


def _kernel(q_hbm, k_hbm, v_hbm, s_hbm, w1_hbm, w3_hbm, w2_hbm, wm_hbm, sh_hbm, dd_hbm, c_hbm, f_hbm, g_hbm,
            out_hbm,
            q_v, k_v, v_v, s_v, w1_v, w3_v, w2_v, wm_v, sh_v, dd_v, cc_v, f_v, g_v, one_v,
            f2_v, g2_v, s2_v, kv_v, u_v, w_v, c_v, y_v, z_v, h_v, n_v, act0_v, act1_v, out_v, mod_v,
            sems):
    f32, bf16 = jnp.float32, jnp.bfloat16
    n_sem = [0]

    def cp(src, dst):
        n_sem[0] += 1
        return pltpu.make_async_copy(src, dst, sems.at[n_sem[0] - 1])

    def wait(copies):
        for c in copies:
            c.wait()

    def rows(j, n):
        return pl.ds(j * n, n)

    small = [cp(a, b) for a, b in (
        (sh_hbm, sh_v), (f_hbm.at[0:16], one_v), (f_hbm, f_v), (dd_hbm, dd_v), (g_hbm, g_v), (c_hbm, cc_v))]
    kvs = [[cp(k_hbm.at[rows(j, CH)], k_v.at[rows(j, CH)]),
            cp(v_hbm.at[rows(j, CH)], v_v.at[rows(j, CH)]),
            cp(s_hbm.at[:, rows(j, CH)], s_v.at[:, rows(j, CH)])] for j in range(NCH)]
    wm = {j: cp(wm_hbm.at[:, rows(j, D)], wm_v.at[:, rows(j, D)]) for j in range(6)}
    qc = [cp(q_hbm.at[rows(t, TM)], q_v.at[rows(t, TM)]) for t in range(NT)]
    w13 = [[cp(w1_hbm.at[:, rows(j, FC)], w1_v.at[:, rows(j, FC)]),
            cp(w3_hbm.at[:, rows(j, FC)], w3_v.at[:, rows(j, FC)])] for j in range(NF)]
    w2c = cp(w2_hbm, w2_v)
    oc = [[cp(out_v.at[rows(t, TM)], out_hbm.at[rows(t, TM)])] for t in range(NT - 1)]
    oc.append([cp(out_v.at[pl.ds(S - TM + r, n)], out_hbm.at[pl.ds(S - TM + r, n)]) for r, n in LAST_PARTS])

    need = [small[:2] + kvs[0][:2], kvs[0][2:] + small[2:4] + kvs[1][:2]]
    need += [kvs[j - 1][2:] + kvs[j][:2] for j in range(2, NCH - 1)] + [kvs[NCH - 2][2:] + kvs[NCH - 1][2:]]
    need[NCH - 2] += kvs[NCH - 1][:2]
    need[2] += small[4:]
    queue = [c for cs in need for c in cs]
    queue += [wm[2], wm[1], wm[0], qc[0], wm[4], wm[3], qc[1]] + w13[0]
    queue += [c for j in range(1, NF) for c in w13[j]] + [qc[2], wm[5], w2c] + qc[3:]
    for c in queue:
        c.start()

    def gate(r0):
        sh = sh_v[...].astype(f32)
        kb = after(k_v[pl.ds(r0, KR), :], chain.get(0)).astype(f32)
        prev = jnp.zeros((8, D), f32) if r0 == 0 else k_v[pl.ds(r0 - 16, 16), :].astype(f32)[8:]
        kk = jnp.concatenate([prev, kb], axis=0)
        ks = kb * sh[0:1]
        for j in range(1, 4):
            ks = ks + pltpu.roll(kk, j, 0)[8:] * sh[j:j + 1]
        kv = (ks * v_v[pl.ds(r0, KR), :].astype(f32)).astype(bf16)
        kv_v[pl.ds(r0, KR), :] = kv
        link(0, bits(kv))

    def fwd_signal(b):
        u = jnp.dot(f2_v[:2 * L], kv_v[rows(b, L), :], preferred_element_type=f32).reshape(NG, 2, 8, D)
        u_v[b] = jnp.stack([u[:, 0] + u[:, 1], u[:, 0], u[:, 1]], axis=1).reshape(3 * L, D)

    def fwd_filter(b):
        w = lax.dot_general(f2_v[2 * L:], s2_v[:, rows(b, L)], (((1,), (1,)), ((), ())), preferred_element_type=f32)
        w = w.reshape(NG, 2, 8, D)
        if b == 0:
            dd = dd_v[...].astype(f32).reshape(1, 1, D)
            cq, cr = w[:, 0] - dd, w[:, 1] + dd
            w = jnp.stack([cq, cr], axis=1)
        else:
            p = w_v[(b - 1) % 2].reshape(NG, 2, 8, D)
            H = NG // 2
            cq = jnp.concatenate([w[:H, 0] + p[:H, 1], w[H:, 0] - p[H:, 1]], axis=0)
            cr = jnp.concatenate([w[:H, 1] - p[:H, 0], w[H:, 1] + p[H:, 0]], axis=0)
        c_v[b] = jnp.stack([cr - cq, cq, cr], axis=1).reshape(3 * L, D)
        if b + 1 < NB:
            w_v[b % 2] = w.reshape(2 * L, D)

    def always():
        return bits(one_v[...]) != jnp.uint32(0xFFFFFFFF)

    def bits(x):
        return pltpu.bitcast(x, jnp.uint32)

    def fold(x, n):
        parts = [x[r:r + 8, c:c + 128] for r in range(0, x.shape[0], 8) for c in range(0, x.shape[1], 128)]
        outs = [functools.reduce(jnp.bitwise_or, parts[i::n]) for i in range(n)]
        return outs[0] if n == 1 else jnp.concatenate(outs, axis=1)

    def after(x, dep):
        if dep is None:
            return x
        xi = bits(x)
        reps = (xi.shape[0] // 8, xi.shape[1] // 128)
        if dep.shape != xi.shape:
            dep = jnp.tile(fold(dep, 1), reps)
        return pltpu.bitcast(jnp.where(jnp.tile(always(), reps), xi, dep), x.dtype)

    chain = {}

    def link(key, dep):
        dep = fold(dep, 1)
        chain[key] = dep

    def mac(outs, l, g, parts):
        ls = pl.ds(l * 128, 128)
        acc = {}
        for part in parts:
            for m in range(max(outs) + 1):
                for i in part:
                    rs = pl.ds(g * 24 + i * 8, 8)
                    c = c_v[m, rs, ls]
                    if m == 0:
                        c = after(c, chain.get(0))
                    for a in outs:
                        if m <= a:
                            t = c * u_v[a - m, rs, ls]
                            acc[a, i] = t if m == 0 else acc[a, i] + t
            if part is not parts[-1]:
                link(0, jnp.concatenate([bits(acc[a, i]) for a in outs for i in part], axis=1))
        ys = []
        for a in outs:
            k0 = 0.5 * acc[a, 0]
            y = jnp.concatenate([k0 - acc[a, 2], k0 + acc[a, 1]], axis=0).astype(bf16)
            y_v[pl.ds(a * 2 * L + g * 16, 16), ls] = y
            ys.append(bits(y))
        link(0, jnp.concatenate(ys, axis=1))

    def mod(j):
        cc = cc_v[...].astype(f32)
        sc = jnp.broadcast_to(cc * jax.nn.sigmoid(cc), (16, D)).astype(bf16)
        m = jnp.dot(sc, wm_v[:, rows(j, D)], preferred_element_type=f32)[:8]
        if j in (1, 4):
            m = 1 + m
        if j in (0, 1):
            m = m * mod_v[2]
        mod_v[j] = m

    def ln(r0, key):
        rs = pl.ds(r0, LNR)
        sa, ca, sb, cb = [jnp.tile(mod_v[j], (LNR // 8, 1)) for j in (0, 1, 3, 4)]
        x = after(q_v[rs, :], chain.get(key)).astype(f32)
        x1 = x + (_norm(x) * ca + sa) * z_v[rs, :]
        z_v[rs, :] = x1
        h = (_norm(x1) * cb + sb).astype(bf16)
        h_v[rs, :] = h
        link(key, bits(h))

    def ln_first_a(r0):
        rs = pl.ds(r0, LNR)
        sa, ca = [jnp.tile(mod_v[j], (LNR // 8, 1)) for j in range(2)]
        x = q_v[rs, :].astype(f32)
        x1 = x + (_norm(x) * ca + sa) * z_v[rs, :]
        z_v[rs, :] = x1
        n_v[rs, :] = _norm(x1)

    def ln_first_b(r0):
        rs = pl.ds(r0, LNR)
        sb, cb = [jnp.tile(mod_v[j], (LNR // 8, 1)) for j in (3, 4)]
        h_v[rs, :] = (n_v[rs, :] * cb + sb).astype(bf16)

    def up(t, j):
        h = h_v[rows(t, TM), :]
        w1, w3 = w1_v[:, rows(j, FC)], w3_v[:, rows(j, FC)]
        g = 0.5 * jnp.dot(h, w1, preferred_element_type=f32)
        u = jnp.dot(h, w3, preferred_element_type=f32)
        (act0_v, act1_v)[t % 2][:, rows(j, FC)] = ((g * jnp.tanh(g) + g) * u).astype(bf16)

    def down(t):
        w2 = w2_v[...]
        for c, (r, n) in zip(oc[t], LAST_PARTS if t == NT - 1 else ((0, TM),)):
            o = jnp.dot((act0_v, act1_v)[t % 2][pl.ds(r, n), :], w2, preferred_element_type=f32)
            rs = pl.ds(t * TM + r, n)
            out_v[rs, :] = (z_v[rs, :] + jnp.tile(mod_v[5], (n // 8, 1)) * o).astype(bf16)
            c.start()

    def run(tasks):
        for kind, j, *rest in tasks:
            if kind == "gate":
                for r0 in range(j * CH, (j + 1) * CH, KR):
                    gate(r0)
            elif kind == "fw":
                s2_v[:, rows(j, CH)] = s_v[:, rows(j, CH)]
                fwd_filter(2 * j)
                fwd_filter(2 * j + 1)
            elif kind == "fu":
                fwd_signal(2 * j)
                fwd_signal(2 * j + 1)
            elif kind == "inv":
                ls = pl.ds(rest[0][0] * 128, len(rest[0]) * 128)
                for b in (2 * j, 2 * j + 1):
                    z_v[rows(b, L), ls] = jnp.dot(g2_v[...], y_v[rows(b, 2 * L), ls], preferred_element_type=f32)
            else:
                parts = ((0,), (1,), (2,)) if rest[1:] else ((0, 1, 2),)
                for l in rest[0]:
                    for g in range(NG):
                        mac((2 * j, 2 * j + 1), l, g, parts)

    for j, tasks in enumerate(PROLOGUE):
        wait(need[j])
        if j == 1:
            f2_v[...] = f_v[...]
        if j == 2:
            g2_v[...] = g_v[...]
        chain.clear()
        run(tasks)

    wait((wm[2], wm[1], wm[0], qc[0], wm[4], wm[3]))
    chain.clear()
    for j in (2, 1, 0):
        mod(j)
    for r0 in range(0, TM, LNR):
        ln_first_a(r0)
    for j in (4, 3):
        mod(j)
    for r0 in range(0, TM, LNR):
        ln_first_b(r0)

    for j in range(3):
        wait(w13[j] + ([qc[1]] if j == 0 else []))
        chain.clear()
        for i, r0 in enumerate(range(LN1_CUTS[j], LN1_CUTS[j + 1], LNR)):
            ln(TM + r0, "ln%d" % (i % 3))
        up(0, j)
    for j in range(3):
        up(1, j)
    wait(w13[3] + w13[4] + w13[5] + [qc[2]])
    chain.clear()
    for r0 in range(0, TM // 2, LNR):
        ln(2 * TM + r0, "ln")
    for j in range(3, NF):
        up(0, j)
        up(1, j)
    wait([wm[5], w2c, qc[3]])
    mod(5)
    chain.clear()
    for r0 in range(TM // 2, TM, LNR):
        ln(2 * TM + r0, "ln")
    down(0)
    down(1)

    def late(*pos):
        if pos in LATE:
            chain.pop(0, None)
            run(LATE[pos])

    for t in range(2, NT):
        if 3 <= t < NT - 1:
            wait(oc[t - 3] + (qc[4:] if t == 3 else []))
            chain.clear()
        for j in range(NF):
            late(t, j)
            if j == 0 and t + 1 < NT:
                for r0 in range((t + 1) * TM, (t + 2) * TM, LNR):
                    ln(r0, "ln")
            up(t, j)
        late(t, NF)
        down(t)
    wait([c for cs in oc[NT - 4:] for c in cs])


def pallas_adaLN_cond__ssm_conv_h3__glu_gated_swiglu__prompt_kernel(
        A_q, A_k, A_v, A_shift_k, A_ssm_k, A_ssm_D, B_x, B_w1, B_w3, B_w2, c, w_mod):
    Fm, Gm = _dft_mats()
    f32, bf16 = jnp.float32, jnp.bfloat16
    anyspec = pl.BlockSpec(memory_space=pl.ANY)
    V = pltpu.VMEM
    dma = pltpu.SemaphoreType.DMA
    out = pl.pallas_call(
        _kernel,
        in_specs=[anyspec] * 13,
        out_specs=anyspec,
        out_shape=jax.ShapeDtypeStruct((S, D), bf16),
        scratch_shapes=[
            V((S, D), bf16), V((S, D), bf16), V((S, D), bf16), V((D, S), bf16),
            V((D, FF), bf16), V((D, FF), bf16), V((FF, D), bf16), V((D, 6 * D), bf16),
            V((4, D), bf16), V((D,), bf16), V((1, D), bf16), V((4 * L, L), bf16), V((L, 2 * L), bf16), V((16, L), bf16),
            V((4 * L, L), bf16), V((L, 2 * L), bf16), V((D, S), bf16),
            V((S, D), bf16), V((NB, 3 * L, D), f32), V((2, 2 * L, D), f32), V((NB, 3 * L, D), f32), V((NB * 2 * L, D), bf16),
            V((S, D), f32), V((S, D), bf16), V((TM, D), f32), V((TM, FF), bf16), V((TM, FF), bf16), V((S, D), bf16), V((6, 8, D), f32),
            dma((N_COPIES,)),
        ],
        compiler_params=pltpu.CompilerParams(vmem_limit_bytes=110 * 1024 * 1024),
    )(A_q.reshape(S, D), A_k.reshape(S, D), A_v.reshape(S, D), A_ssm_k, B_w1, B_w3, B_w2, w_mod,
      A_shift_k.T, A_ssm_D, c, Fm, Gm)
    return out.reshape(1, S, D)
```

```python
import functools
import numpy as np
import jax
import jax.numpy as jnp
from jax import lax
import jax.experimental.pallas as pl
import jax.experimental.pallas.tpu as pltpu

S, D, FF = 2048, 640, 1536
EPS = 1e-5
L = 128
NB = S // L
NG = L // 8
NL = D // 128
CH = 2 * L
NCH = S // CH
TM = 256
NT = S // TM
FC = 256
NF = FF // FC
KR = 32
LNR = 16
ALL = range(NL)

PROLOGUE = (
    (("gate", 0),),
    (("fu", 0), ("fw", 0), ("gate", 1)),
    (("fu", 1), ("fw", 1), ("mac", 0, ALL), ("inv", 0, ALL), ("gate", 2)),
    (("fu", 2), ("fw", 2), ("mac", 1, ALL), ("inv", 1, ALL), ("gate", 3)),
    (("fu", 3), ("fw", 3), ("mac", 2, (0, 1, 2, 3)), ("inv", 2, (0, 1, 2, 3)), ("gate", 4)),
    (("fu", 4), ("fw", 4), ("mac", 2, (4,)), ("mac", 3, (0, 1)), ("inv", 2, (4,)), ("inv", 3, (0, 1)), ("gate", 5)),
    (("fu", 5), ("fw", 5), ("mac", 3, (2, 3, 4)), ("inv", 3, (2, 3, 4)), ("gate", 6), ("gate", 7)),
    (("fu", 6), ("fw", 6), ("fu", 7), ("fw", 7)),
)
LATE = {
    (2, NF): (("mac", 4, ALL, True), ("mac", 5, ALL, True)),
    (3, 0): (("inv", 4, ALL), ("inv", 5, ALL)),
    (4, NF): (("mac", 6, ALL, True), ("mac", 7, ALL, True)),
    (5, 0): (("inv", 6, ALL), ("inv", 7, ALL)),
}
LN1_CUTS = (0, 96, 192, 256)
LAST_PARTS = ((0, 192), (192, 64))
N_COPIES = 6 + 3 * NCH + 6 + NT + 2 * NF + 1 + (NT - 1) + len(LAST_PARTS)


def _dft_mats():
    ks = np.concatenate([np.arange(0, L, 2), np.arange(1, L, 2)])
    th = 2 * np.pi * (ks + 0.5) / (2 * L)
    j = np.arange(L)
    ang = (th[:, None] * j[None, :]).reshape(L // 8, 1, 8, L)
    Fm = np.concatenate([np.cos(ang), -np.sin(ang)], 1).reshape(2 * L, L)
    Gm = Fm.T / L
    Hm = np.concatenate([-np.sin(ang) - np.cos(ang), np.cos(ang) - np.sin(ang)], 1).reshape(2 * L, L)
    return (np.concatenate([Fm, Hm], 0).astype(jnp.bfloat16), np.ascontiguousarray(Gm).astype(jnp.bfloat16))


def _norm(x):
    m = jnp.sum(x, axis=-1, keepdims=True) * (1.0 / D)
    xc = x - m
    v = jnp.sum(xc * xc, axis=-1, keepdims=True) * (1.0 / D)
    return xc * lax.rsqrt(v + EPS)


def _kernel(q_hbm, k_hbm, v_hbm, s_hbm, w1_hbm, w3_hbm, w2_hbm, wm_hbm, sh_hbm, dd_hbm, c_hbm, f_hbm, g_hbm,
            out_hbm,
            q_v, k_v, v_v, s_v, w1_v, w3_v, w2_v, wm_v, sh_v, dd_v, cc_v, f_v, g_v, one_v,
            f2_v, g2_v, kv_v, u_v, w_v, c_v, y_v, z_v, h_v, n_v, act0_v, act1_v, out_v, mod_v,
            sems):
    f32, bf16 = jnp.float32, jnp.bfloat16
    n_sem = [0]

    def cp(src, dst):
        n_sem[0] += 1
        return pltpu.make_async_copy(src, dst, sems.at[n_sem[0] - 1])

    def wait(copies):
        for c in copies:
            c.wait()

    def rows(j, n):
        return pl.ds(j * n, n)

    small = [cp(a, b) for a, b in (
        (sh_hbm, sh_v), (f_hbm.at[0:16], one_v), (f_hbm, f_v), (dd_hbm, dd_v), (g_hbm, g_v), (c_hbm, cc_v))]
    kvs = [[cp(k_hbm.at[rows(j, CH)], k_v.at[rows(j, CH)]),
            cp(v_hbm.at[rows(j, CH)], v_v.at[rows(j, CH)]),
            cp(s_hbm.at[:, rows(j, CH)], s_v.at[:, rows(j, CH)])] for j in range(NCH)]
    wm = {j: cp(wm_hbm.at[:, rows(j, D)], wm_v.at[:, rows(j, D)]) for j in range(6)}
    qc = [cp(q_hbm.at[rows(t, TM)], q_v.at[rows(t, TM)]) for t in range(NT)]
    w13 = [[cp(w1_hbm.at[:, rows(j, FC)], w1_v.at[:, rows(j, FC)]),
            cp(w3_hbm.at[:, rows(j, FC)], w3_v.at[:, rows(j, FC)])] for j in range(NF)]
    w2c = cp(w2_hbm, w2_v)
    oc = [[cp(out_v.at[rows(t, TM)], out_hbm.at[rows(t, TM)])] for t in range(NT - 1)]
    oc.append([cp(out_v.at[pl.ds(S - TM + r, n)], out_hbm.at[pl.ds(S - TM + r, n)]) for r, n in LAST_PARTS])

    need = [small[:2] + kvs[0][:2], kvs[0][2:] + small[2:4] + kvs[1][:2]]
    need += [kvs[j - 1][2:] + kvs[j][:2] for j in range(2, NCH - 1)] + [kvs[NCH - 2][2:] + kvs[NCH - 1][2:]]
    need[NCH - 2] += kvs[NCH - 1][:2]
    need[2] += small[4:]
    queue = [c for cs in need for c in cs]
    queue += [wm[2], wm[1], wm[0], qc[0], wm[4], wm[3], qc[1]] + w13[0]
    queue += [c for j in range(1, NF) for c in w13[j]] + [qc[2], wm[5], w2c] + qc[3:]
    for c in queue:
        c.start()

    def gate(r0):
        sh = sh_v[...].astype(f32)
        kb = after(k_v[pl.ds(r0, KR), :], chain.get(0)).astype(f32)
        prev = jnp.zeros((8, D), f32) if r0 == 0 else k_v[pl.ds(r0 - 16, 16), :].astype(f32)[8:]
        kk = jnp.concatenate([prev, kb], axis=0)
        ks = kb * sh[0:1]
        for j in range(1, 4):
            ks = ks + pltpu.roll(kk, j, 0)[8:] * sh[j:j + 1]
        kv = (ks * v_v[pl.ds(r0, KR), :].astype(f32)).astype(bf16)
        kv_v[pl.ds(r0, KR), :] = kv
        link(0, bits(kv))

    def fwd_signal(b):
        u = jnp.dot(f2_v[:2 * L], kv_v[rows(b, L), :], preferred_element_type=f32)
        u_v[b] = u

    def fwd_filter(b):
        w = lax.dot_general(f2_v[2 * L:], s_v[:, rows(b, L)], (((1,), (1,)), ((), ())), preferred_element_type=f32)
        w = w.reshape(NG, 2, 8, D)
        if b == 0:
            dd = dd_v[...].astype(f32).reshape(1, 1, D)
            cq, cr = w[:, 0] - dd, w[:, 1] + dd
            w = jnp.stack([cq, cr], axis=1)
        else:
            p = w_v[(b - 1) % 2].reshape(NG, 2, 8, D)
            H = NG // 2
            cq = jnp.concatenate([w[:H, 0] + p[:H, 1], w[H:, 0] - p[H:, 1]], axis=0)
            cr = jnp.concatenate([w[:H, 1] - p[:H, 0], w[H:, 1] + p[H:, 0]], axis=0)
        c_v[b] = jnp.stack([cq, cr], axis=1).reshape(2 * L, D)
        if b + 1 < NB:
            w_v[b % 2] = w.reshape(2 * L, D)

    def always():
        return bits(one_v[...]) != jnp.uint32(0xFFFFFFFF)

    def bits(x):
        return pltpu.bitcast(x, jnp.uint32)

    def fold(x, n):
        parts = [x[r:r + 8, c:c + 128] for r in range(0, x.shape[0], 8) for c in range(0, x.shape[1], 128)]
        outs = [functools.reduce(jnp.bitwise_or, parts[i::n]) for i in range(n)]
        return outs[0] if n == 1 else jnp.concatenate(outs, axis=1)

    def after(x, dep):
        if dep is None:
            return x
        xi = bits(x)
        reps = (xi.shape[0] // 8, xi.shape[1] // 128)
        if dep.shape != xi.shape:
            dep = jnp.tile(fold(dep, 1), reps)
        return pltpu.bitcast(jnp.where(jnp.tile(always(), reps), xi, dep), x.dtype)

    chain = {}

    def link(key, dep):
        dep = fold(dep, 1)
        chain[key] = dep

    def mac(outs, l, g, parts):
        ls = pl.ds(l * 128, 128)
        acc = {}

        def signal(b, i):
            if i == 0:
                return signal(b, 1) + signal(b, 2)
            return u_v[b, pl.ds(g * 16 + (i - 1) * 8, 8), ls]

        for part in parts:
            for m in range(max(outs) + 1):
                for i in part:
                    cq, cr = pl.ds(g * 16, 8), pl.ds(g * 16 + 8, 8)
                    c = c_v[m, cr, ls] - c_v[m, cq, ls] if i == 0 else c_v[m, cq if i == 1 else cr, ls]
                    if m == 0:
                        c = after(c, chain.get(0))
                    for a in outs:
                        if m <= a:
                            t = c * signal(a - m, i)
                            acc[a, i] = t if m == 0 else acc[a, i] + t
            if part is not parts[-1]:
                link(0, jnp.concatenate([bits(acc[a, i]) for a in outs for i in part], axis=1))
        ys = []
        for a in outs:
            k0 = 0.5 * acc[a, 0]
            y = jnp.concatenate([k0 - acc[a, 2], k0 + acc[a, 1]], axis=0).astype(bf16)
            y_v[pl.ds(a * 2 * L + g * 16, 16), ls] = y
            ys.append(bits(y))
        link(0, jnp.concatenate(ys, axis=1))

    def mod(j):
        cc = cc_v[...].astype(f32)
        sc = jnp.broadcast_to(cc * jax.nn.sigmoid(cc), (16, D)).astype(bf16)
        m = jnp.dot(sc, wm_v[:, rows(j, D)], preferred_element_type=f32)[:8]
        if j in (1, 4):
            m = 1 + m
        if j in (0, 1):
            m = m * mod_v[2]
        mod_v[j] = m

    def ln(r0, key):
        rs = pl.ds(r0, LNR)
        sa, ca, sb, cb = [jnp.tile(mod_v[j], (LNR // 8, 1)) for j in (0, 1, 3, 4)]
        x = after(q_v[rs, :], chain.get(key)).astype(f32)
        x1 = x + (_norm(x) * ca + sa) * z_v[rs, :]
        z_v[rs, :] = x1
        h = (_norm(x1) * cb + sb).astype(bf16)
        h_v[rs, :] = h
        link(key, bits(h))

    def ln_first_a(r0):
        rs = pl.ds(r0, LNR)
        sa, ca = [jnp.tile(mod_v[j], (LNR // 8, 1)) for j in range(2)]
        x = q_v[rs, :].astype(f32)
        x1 = x + (_norm(x) * ca + sa) * z_v[rs, :]
        z_v[rs, :] = x1
        n_v[rs, :] = _norm(x1)

    def ln_first_b(r0):
        rs = pl.ds(r0, LNR)
        sb, cb = [jnp.tile(mod_v[j], (LNR // 8, 1)) for j in (3, 4)]
        h_v[rs, :] = (n_v[rs, :] * cb + sb).astype(bf16)

    def up(t, j):
        h = h_v[rows(t, TM), :]
        w1, w3 = w1_v[:, rows(j, FC)], w3_v[:, rows(j, FC)]
        g = 0.5 * jnp.dot(h, w1, preferred_element_type=f32)
        u = jnp.dot(h, w3, preferred_element_type=f32)
        (act0_v, act1_v)[t % 2][:, rows(j, FC)] = ((g * jnp.tanh(g) + g) * u).astype(bf16)

    def down(t):
        w2 = w2_v[...]
        for c, (r, n) in zip(oc[t], LAST_PARTS if t == NT - 1 else ((0, TM),)):
            o = jnp.dot((act0_v, act1_v)[t % 2][pl.ds(r, n), :], w2, preferred_element_type=f32)
            rs = pl.ds(t * TM + r, n)
            out_v[rs, :] = (z_v[rs, :] + jnp.tile(mod_v[5], (n // 8, 1)) * o).astype(bf16)
            c.start()

    def run(tasks):
        for kind, j, *rest in tasks:
            if kind == "gate":
                for r0 in range(j * CH, (j + 1) * CH, KR):
                    gate(r0)
            elif kind == "fw":
                fwd_filter(2 * j)
                fwd_filter(2 * j + 1)
            elif kind == "fu":
                fwd_signal(2 * j)
                fwd_signal(2 * j + 1)
            elif kind == "inv":
                ls = pl.ds(rest[0][0] * 128, len(rest[0]) * 128)
                for b in (2 * j, 2 * j + 1):
                    z_v[rows(b, L), ls] = jnp.dot(g2_v[...], y_v[rows(b, 2 * L), ls], preferred_element_type=f32)
            else:
                parts = ((0,), (1,), (2,)) if rest[1:] else ((0, 1, 2),)
                for l in rest[0]:
                    for g in range(NG):
                        mac((2 * j, 2 * j + 1), l, g, parts)

    for j, tasks in enumerate(PROLOGUE):
        wait(need[j])
        if j == 1:
            f2_v[...] = f_v[...]
        if j == 2:
            g2_v[...] = g_v[...]
        chain.clear()
        run(tasks)

    wait((wm[2], wm[1], wm[0], qc[0], wm[4], wm[3]))
    chain.clear()
    for j in (2, 1, 0):
        mod(j)
    for r0 in range(0, TM, LNR):
        ln_first_a(r0)
    for j in (4, 3):
        mod(j)
    for r0 in range(0, TM, LNR):
        ln_first_b(r0)

    for j in range(3):
        wait(w13[j] + ([qc[1]] if j == 0 else []))
        chain.clear()
        for i, r0 in enumerate(range(LN1_CUTS[j], LN1_CUTS[j + 1], LNR)):
            ln(TM + r0, "ln%d" % (i % 3))
        up(0, j)
    for j in range(3):
        up(1, j)
    wait(w13[3] + w13[4] + w13[5] + [qc[2]])
    chain.clear()
    for r0 in range(0, TM // 2, LNR):
        ln(2 * TM + r0, "ln")
    for j in range(3, NF):
        up(0, j)
        up(1, j)
    wait([wm[5], w2c, qc[3]])
    mod(5)
    chain.clear()
    for r0 in range(TM // 2, TM, LNR):
        ln(2 * TM + r0, "ln")
    down(0)
    down(1)

    def late(*pos):
        if pos in LATE:
            chain.pop(0, None)
            run(LATE[pos])

    for t in range(2, NT):
        if t in (3, 5):
            wait(oc[(t - 3) // 2] + (qc[4:] if t == 3 else []))
            chain.clear()
        for j in range(NF):
            late(t, j)
            if j == 0 and t + 1 < NT:
                for r0 in range((t + 1) * TM, (t + 2) * TM, LNR):
                    ln(r0, "ln")
            up(t, j)
        late(t, NF)
        down(t)
    wait([c for cs in oc[2:] for c in cs])


def pallas_adaLN_cond__ssm_conv_h3__glu_gated_swiglu__prompt_kernel(
        A_q, A_k, A_v, A_shift_k, A_ssm_k, A_ssm_D, B_x, B_w1, B_w3, B_w2, c, w_mod):
    Fm, Gm = _dft_mats()
    f32, bf16 = jnp.float32, jnp.bfloat16
    anyspec = pl.BlockSpec(memory_space=pl.ANY)
    V = pltpu.VMEM
    dma = pltpu.SemaphoreType.DMA
    out = pl.pallas_call(
        _kernel,
        in_specs=[anyspec] * 13,
        out_specs=anyspec,
        out_shape=jax.ShapeDtypeStruct((S, D), bf16),
        scratch_shapes=[
            V((S, D), bf16), V((S, D), bf16), V((S, D), bf16), V((D, S), bf16),
            V((D, FF), bf16), V((D, FF), bf16), V((FF, D), bf16), V((D, 6 * D), bf16),
            V((4, D), bf16), V((D,), bf16), V((1, D), bf16), V((4 * L, L), bf16), V((L, 2 * L), bf16), V((16, L), bf16),
            V((4 * L, L), bf16), V((L, 2 * L), bf16),
            V((S, D), bf16), V((NB, 2 * L, D), f32), V((2, 2 * L, D), f32), V((NB, 2 * L, D), f32), V((NB * 2 * L, D), bf16),
            V((S, D), f32), V((S, D), bf16), V((TM, D), f32), V((TM, FF), bf16), V((TM, FF), bf16), V((S, D), bf16), V((6, 8, D), f32),
            dma((N_COPIES,)),
        ],
        compiler_params=pltpu.CompilerParams(vmem_limit_bytes=110 * 1024 * 1024),
    )(A_q.reshape(S, D), A_k.reshape(S, D), A_v.reshape(S, D), A_ssm_k, B_w1, B_w3, B_w2, w_mod,
      A_shift_k.T, A_ssm_D, c, Fm, Gm)
    return out.reshape(1, S, D)
```

```python
import functools
import numpy as np
import jax
import jax.numpy as jnp
from jax import lax
import jax.experimental.pallas as pl
import jax.experimental.pallas.tpu as pltpu

S, D, FF = 2048, 640, 1536
EPS = 1e-5
L = 128
NB = S // L
NG = L // 8
NL = D // 128
CH = 2 * L
NCH = S // CH
TM = 256
NT = S // TM
FC = 256
NF = FF // FC
KR = 32
LNR = 16
ALL = range(NL)

PROLOGUE = (
    (("gate", 0),),
    (("fu", 0), ("fw", 0)),
    (("gate", 1),),
    (("fu", 1), ("fw", 1), ("mac", 0, ALL), ("inv", 0, ALL)),
    (("gate", 2),),
    (("fu", 2), ("fw", 2), ("mac", 1, ALL), ("inv", 1, ALL), ("gate", 3)),
    (("fu", 3), ("fw", 3), ("mac", 2, (0, 1, 2, 3)), ("inv", 2, (0, 1, 2, 3)), ("gate", 4)),
    (("fu", 4), ("fw", 4), ("mac", 2, (4,)), ("mac", 3, (0, 1)), ("inv", 2, (4,)), ("inv", 3, (0, 1)), ("gate", 5)),
    (("fu", 5), ("fw", 5), ("mac", 3, (2, 3, 4)), ("inv", 3, (2, 3, 4)), ("gate", 6), ("gate", 7)),
    (("fu", 6), ("fw", 6), ("fu", 7), ("fw", 7), ("mac", 4, ALL), ("inv", 4, ALL)),
)
LATE = {
    (2, NF): (("mac", 5, ALL, True), ("mac", 6, (0, 1), True)),
    (3, 0): (("inv", 5, ALL),),
    (4, NF): (("mac", 6, (2, 3, 4), True), ("mac", 7, ALL, True)),
    (5, 0): (("inv", 6, ALL), ("inv", 7, ALL)),
}
LN1_CUTS = (0, 96, 192, 256)
LAST_PARTS = ((0, 192), (192, 64))
N_COPIES = 6 + 3 * NCH + 6 + NT + 2 * NF + 1 + (NT - 1) + len(LAST_PARTS)


def _dft_mats():
    ks = np.concatenate([np.arange(0, L, 2), np.arange(1, L, 2)])
    th = 2 * np.pi * (ks + 0.5) / (2 * L)
    j = np.arange(L)
    ang = (th[:, None] * j[None, :]).reshape(L // 8, 1, 8, L)
    Fm = np.concatenate([np.cos(ang), -np.sin(ang)], 1).reshape(2 * L, L)
    Gm = Fm.T / L
    Hm = np.concatenate([-np.sin(ang) - np.cos(ang), np.cos(ang) - np.sin(ang)], 1).reshape(2 * L, L)
    return (np.concatenate([Fm, Hm], 0).astype(jnp.bfloat16), np.ascontiguousarray(Gm).astype(jnp.bfloat16))


def _norm(x):
    m = jnp.sum(x, axis=-1, keepdims=True) * (1.0 / D)
    xc = x - m
    v = jnp.sum(xc * xc, axis=-1, keepdims=True) * (1.0 / D)
    return xc * lax.rsqrt(v + EPS)


def _kernel(q_hbm, k_hbm, v_hbm, s_hbm, w1_hbm, w3_hbm, w2_hbm, wm_hbm, sh_hbm, dd_hbm, c_hbm, f_hbm, g_hbm,
            out_hbm,
            q_v, k_v, v_v, s_v, w1_v, w3_v, w2_v, wm_v, sh_v, dd_v, cc_v, f_v, g_v, one_v,
            f2_v, g2_v, kv_v, u_v, w_v, c_v, y_v, z_v, h_v, n_v, act0_v, act1_v, out_v, mod_v,
            sems):
    f32, bf16 = jnp.float32, jnp.bfloat16
    n_sem = [0]

    def cp(src, dst):
        n_sem[0] += 1
        return pltpu.make_async_copy(src, dst, sems.at[n_sem[0] - 1])

    def wait(copies):
        for c in copies:
            c.wait()

    def rows(j, n):
        return pl.ds(j * n, n)

    small = [cp(a, b) for a, b in (
        (sh_hbm, sh_v), (f_hbm.at[0:16], one_v), (f_hbm, f_v), (dd_hbm, dd_v), (g_hbm, g_v), (c_hbm, cc_v))]
    kvs = [[cp(k_hbm.at[rows(j, CH)], k_v.at[rows(j, CH)]),
            cp(v_hbm.at[rows(j, CH)], v_v.at[rows(j, CH)]),
            cp(s_hbm.at[:, rows(j, CH)], s_v.at[:, rows(j, CH)])] for j in range(NCH)]
    wm = {j: cp(wm_hbm.at[:, rows(j, D)], wm_v.at[:, rows(j, D)]) for j in range(6)}
    qc = [cp(q_hbm.at[rows(t, TM)], q_v.at[rows(t, TM)]) for t in range(NT)]
    w13 = [[cp(w1_hbm.at[:, rows(j, FC)], w1_v.at[:, rows(j, FC)]),
            cp(w3_hbm.at[:, rows(j, FC)], w3_v.at[:, rows(j, FC)])] for j in range(NF)]
    w2c = cp(w2_hbm, w2_v)
    oc = [[cp(out_v.at[rows(t, TM)], out_hbm.at[rows(t, TM)])] for t in range(NT - 1)]
    oc.append([cp(out_v.at[pl.ds(S - TM + r, n)], out_hbm.at[pl.ds(S - TM + r, n)]) for r, n in LAST_PARTS])

    need = [small[:2] + kvs[0][:2], kvs[0][2:] + small[2:4], kvs[1][:2], kvs[1][2:] + small[4:], kvs[2][:2]]
    need += [kvs[j - 1][2:] + kvs[j][:2] for j in range(3, NCH - 1)] + [kvs[NCH - 2][2:] + kvs[NCH - 1][2:]]
    need[-2] += kvs[NCH - 1][:2]
    queue = [c for cs in need for c in cs]
    queue += [wm[2], wm[1], wm[0], qc[0], wm[4], wm[3], qc[1]] + w13[0]
    queue += [c for j in range(1, NF) for c in w13[j]] + [qc[2], wm[5], w2c] + qc[3:]
    for c in queue:
        c.start()

    def gate(r0):
        sh = sh_v[...].astype(f32)
        kb = after(k_v[pl.ds(r0, KR), :], chain.get(0)).astype(f32)
        prev = jnp.zeros((8, D), f32) if r0 == 0 else k_v[pl.ds(r0 - 16, 16), :].astype(f32)[8:]
        kk = jnp.concatenate([prev, kb], axis=0)
        ks = kb * sh[0:1]
        for j in range(1, 4):
            ks = ks + pltpu.roll(kk, j, 0)[8:] * sh[j:j + 1]
        kv = (ks * v_v[pl.ds(r0, KR), :].astype(f32)).astype(bf16)
        kv_v[pl.ds(r0, KR), :] = kv
        link(0, bits(kv))

    def fwd_signal(b):
        u = jnp.dot(f2_v[:2 * L], kv_v[rows(b, L), :], preferred_element_type=f32)
        u_v[b] = u

    def fwd_filter(b):
        w = lax.dot_general(f2_v[2 * L:], s_v[:, rows(b, L)], (((1,), (1,)), ((), ())), preferred_element_type=f32)
        w = w.reshape(NG, 2, 8, D)
        if b == 0:
            dd = dd_v[...].astype(f32).reshape(1, 1, D)
            cq, cr = w[:, 0] - dd, w[:, 1] + dd
            w = jnp.stack([cq, cr], axis=1)
        else:
            p = w_v[(b - 1) % 2].reshape(NG, 2, 8, D)
            H = NG // 2
            cq = jnp.concatenate([w[:H, 0] + p[:H, 1], w[H:, 0] - p[H:, 1]], axis=0)
            cr = jnp.concatenate([w[:H, 1] - p[:H, 0], w[H:, 1] + p[H:, 0]], axis=0)
        c_v[b] = jnp.stack([cq, cr], axis=1).reshape(2 * L, D)
        if b + 1 < NB:
            w_v[b % 2] = w.reshape(2 * L, D)

    def always():
        return bits(one_v[...]) != jnp.uint32(0xFFFFFFFF)

    def bits(x):
        return pltpu.bitcast(x, jnp.uint32)

    def fold(x, n):
        parts = [x[r:r + 8, c:c + 128] for r in range(0, x.shape[0], 8) for c in range(0, x.shape[1], 128)]
        outs = [functools.reduce(jnp.bitwise_or, parts[i::n]) for i in range(n)]
        return outs[0] if n == 1 else jnp.concatenate(outs, axis=1)

    def after(x, dep):
        if dep is None:
            return x
        xi = bits(x)
        reps = (xi.shape[0] // 8, xi.shape[1] // 128)
        if dep.shape != xi.shape:
            dep = jnp.tile(fold(dep, 1), reps)
        return pltpu.bitcast(jnp.where(jnp.tile(always(), reps), xi, dep), x.dtype)

    chain = {}

    def link(key, dep):
        dep = fold(dep, 1)
        chain[key] = dep

    def mac(outs, l, g, parts):
        ls = pl.ds(l * 128, 128)
        acc = {}

        def signal(b, i):
            if i == 0:
                return signal(b, 1) + signal(b, 2)
            return u_v[b, pl.ds(g * 16 + (i - 1) * 8, 8), ls]

        for part in parts:
            for m in range(max(outs) + 1):
                for i in part:
                    cq, cr = pl.ds(g * 16, 8), pl.ds(g * 16 + 8, 8)
                    c = c_v[m, cr, ls] - c_v[m, cq, ls] if i == 0 else c_v[m, cq if i == 1 else cr, ls]
                    if m == 0:
                        c = after(c, chain.get(0))
                    for a in outs:
                        if m <= a:
                            t = c * signal(a - m, i)
                            acc[a, i] = t if m == 0 else acc[a, i] + t
            if part is not parts[-1]:
                link(0, jnp.concatenate([bits(acc[a, i]) for a in outs for i in part], axis=1))
        ys = []
        for a in outs:
            k0 = 0.5 * acc[a, 0]
            y = jnp.concatenate([k0 - acc[a, 2], k0 + acc[a, 1]], axis=0).astype(bf16)
            y_v[pl.ds(a * 2 * L + g * 16, 16), ls] = y
            ys.append(bits(y))
        link(0, jnp.concatenate(ys, axis=1))

    def mod(j):
        cc = cc_v[...].astype(f32)
        sc = jnp.broadcast_to(cc * jax.nn.sigmoid(cc), (16, D)).astype(bf16)
        m = jnp.dot(sc, wm_v[:, rows(j, D)], preferred_element_type=f32)[:8]
        if j in (1, 4):
            m = 1 + m
        if j in (0, 1):
            m = m * mod_v[2]
        mod_v[j] = m

    def ln(r0, key):
        rs = pl.ds(r0, LNR)
        sa, ca, sb, cb = [jnp.tile(mod_v[j], (LNR // 8, 1)) for j in (0, 1, 3, 4)]
        x = after(q_v[rs, :], chain.get(key)).astype(f32)
        x1 = x + (_norm(x) * ca + sa) * z_v[rs, :]
        z_v[rs, :] = x1
        h = (_norm(x1) * cb + sb).astype(bf16)
        h_v[rs, :] = h
        link(key, bits(h))

    def ln_first_a(r0):
        rs = pl.ds(r0, LNR)
        sa, ca = [jnp.tile(mod_v[j], (LNR // 8, 1)) for j in range(2)]
        x = q_v[rs, :].astype(f32)
        x1 = x + (_norm(x) * ca + sa) * z_v[rs, :]
        z_v[rs, :] = x1
        n_v[rs, :] = _norm(x1)

    def ln_first_b(r0):
        rs = pl.ds(r0, LNR)
        sb, cb = [jnp.tile(mod_v[j], (LNR // 8, 1)) for j in (3, 4)]
        h_v[rs, :] = (n_v[rs, :] * cb + sb).astype(bf16)

    def up(t, j):
        h = h_v[rows(t, TM), :]
        w1, w3 = w1_v[:, rows(j, FC)], w3_v[:, rows(j, FC)]
        g = 0.5 * jnp.dot(h, w1, preferred_element_type=f32)
        u = jnp.dot(h, w3, preferred_element_type=f32)
        (act0_v, act1_v)[t % 2][:, rows(j, FC)] = ((g * jnp.tanh(g) + g) * u).astype(bf16)

    def down(t):
        w2 = w2_v[...]
        for c, (r, n) in zip(oc[t], LAST_PARTS if t == NT - 1 else ((0, TM),)):
            o = jnp.dot((act0_v, act1_v)[t % 2][pl.ds(r, n), :], w2, preferred_element_type=f32)
            rs = pl.ds(t * TM + r, n)
            out_v[rs, :] = (z_v[rs, :] + jnp.tile(mod_v[5], (n // 8, 1)) * o).astype(bf16)
            c.start()

    def run(tasks):
        for kind, j, *rest in tasks:
            if kind == "gate":
                for r0 in range(j * CH, (j + 1) * CH, KR):
                    gate(r0)
            elif kind == "fw":
                fwd_filter(2 * j)
                fwd_filter(2 * j + 1)
            elif kind == "fu":
                fwd_signal(2 * j)
                fwd_signal(2 * j + 1)
            elif kind == "inv":
                ls = pl.ds(rest[0][0] * 128, len(rest[0]) * 128)
                for b in (2 * j, 2 * j + 1):
                    z_v[rows(b, L), ls] = jnp.dot(g2_v[...], y_v[rows(b, 2 * L), ls], preferred_element_type=f32)
            else:
                parts = ((0,), (1,), (2,)) if rest[1:] else ((0, 1, 2),)
                for l in rest[0]:
                    for g in range(NG):
                        mac((2 * j, 2 * j + 1), l, g, parts)

    for j, tasks in enumerate(PROLOGUE):
        wait(need[j])
        if j == 1:
            f2_v[...] = f_v[...]
        if j == 3:
            g2_v[...] = g_v[...]
        chain.clear()
        run(tasks)

    wait((wm[2], wm[1], wm[0], qc[0], wm[4], wm[3]))
    chain.clear()
    for j in (2, 1, 0):
        mod(j)
    for r0 in range(0, TM, LNR):
        ln_first_a(r0)
    for j in (4, 3):
        mod(j)
    for r0 in range(0, TM, LNR):
        ln_first_b(r0)

    for j in range(3):
        wait(w13[j] + ([qc[1]] if j == 0 else []))
        chain.clear()
        for i, r0 in enumerate(range(LN1_CUTS[j], LN1_CUTS[j + 1], LNR)):
            ln(TM + r0, "ln%d" % (i % 3))
        up(0, j)
    for j in range(3):
        up(1, j)
    wait(w13[3] + w13[4] + w13[5] + [qc[2]])
    chain.clear()
    for r0 in range(0, TM // 2, LNR):
        ln(2 * TM + r0, "ln")
    for j in range(3, NF):
        up(0, j)
        up(1, j)
    wait([wm[5], w2c, qc[3]])
    mod(5)
    chain.clear()
    for r0 in range(TM // 2, TM, LNR):
        ln(2 * TM + r0, "ln")
    down(0)
    down(1)

    def late(*pos):
        if pos in LATE:
            chain.pop(0, None)
            run(LATE[pos])

    for t in range(2, NT):
        if t in (3, 5):
            wait(oc[(t - 3) // 2] + (qc[4:] if t == 3 else []))
            chain.clear()
        for j in range(NF):
            late(t, j)
            if j == 0 and t + 1 < NT:
                for r0 in range((t + 1) * TM, (t + 2) * TM, LNR):
                    ln(r0, "ln")
            up(t, j)
        late(t, NF)
        down(t)
    wait([c for cs in oc[2:] for c in cs])


def pallas_adaLN_cond__ssm_conv_h3__glu_gated_swiglu__prompt_kernel(
        A_q, A_k, A_v, A_shift_k, A_ssm_k, A_ssm_D, B_x, B_w1, B_w3, B_w2, c, w_mod):
    Fm, Gm = _dft_mats()
    f32, bf16 = jnp.float32, jnp.bfloat16
    anyspec = pl.BlockSpec(memory_space=pl.ANY)
    V = pltpu.VMEM
    dma = pltpu.SemaphoreType.DMA
    out = pl.pallas_call(
        _kernel,
        in_specs=[anyspec] * 13,
        out_specs=anyspec,
        out_shape=jax.ShapeDtypeStruct((S, D), bf16),
        scratch_shapes=[
            V((S, D), bf16), V((S, D), bf16), V((S, D), bf16), V((D, S), bf16),
            V((D, FF), bf16), V((D, FF), bf16), V((FF, D), bf16), V((D, 6 * D), bf16),
            V((4, D), bf16), V((D,), bf16), V((1, D), bf16), V((4 * L, L), bf16), V((L, 2 * L), bf16), V((16, L), bf16),
            V((4 * L, L), bf16), V((L, 2 * L), bf16),
            V((S, D), bf16), V((NB, 2 * L, D), f32), V((2, 2 * L, D), f32), V((NB, 2 * L, D), f32), V((NB * 2 * L, D), bf16),
            V((S, D), f32), V((S, D), bf16), V((TM, D), f32), V((TM, FF), bf16), V((TM, FF), bf16), V((S, D), bf16), V((6, 8, D), f32),
            dma((N_COPIES,)),
        ],
        compiler_params=pltpu.CompilerParams(vmem_limit_bytes=110 * 1024 * 1024),
    )(A_q.reshape(S, D), A_k.reshape(S, D), A_v.reshape(S, D), A_ssm_k, B_w1, B_w3, B_w2, w_mod,
      A_shift_k.T, A_ssm_D, c, Fm, Gm)
    return out.reshape(1, S, D)
```

```python
import functools
import numpy as np
import jax
import jax.numpy as jnp
from jax import lax
import jax.experimental.pallas as pl
import jax.experimental.pallas.tpu as pltpu

S, D, FF = 2048, 640, 1536
EPS = 1e-5
L = 128
NB = S // L
NG = L // 8
NL = D // 128
CH = 2 * L
NCH = S // CH
TM = 256
NT = S // TM
FC = 256
NF = FF // FC
KR = 32
LNR = 16
ALL = range(NL)

PROLOGUE = (
    (("gate", 0),),
    (("fu", 0), ("fw", 0)),
    (("gate", 1),),
    (("fu", 1), ("fw", 1), ("mac", 0, ALL), ("inv", 0, ALL)),
    (("gate", 2),),
    (("fu", 2), ("fw", 2), ("mac", 1, ALL), ("inv", 1, ALL), ("gate", 3)),
    (("fu", 3), ("fw", 3), ("mac", 2, (0, 1, 2, 3)), ("inv", 2, (0, 1, 2, 3)), ("gate", 4)),
    (("fu", 4), ("fw", 4), ("mac", 2, (4,)), ("mac", 3, (0, 1)), ("inv", 2, (4,)), ("inv", 3, (0, 1)), ("gate", 5)),
    (("fu", 5), ("fw", 5), ("mac", 3, (2, 3, 4)), ("inv", 3, (2, 3, 4)), ("gate", 6), ("gate", 7)),
    (("fu", 6), ("fw", 6), ("fu", 7), ("fw", 7), ("mac", 4, ALL), ("inv", 4, ALL)),
)
LATE = {
    (3, NF): (("mac", 5, ALL, True), ("mac", 6, ALL, True), ("mac", 7, ALL, True)),
    (4, 0): (("inv", 5, ALL), ("inv", 6, ALL), ("inv", 7, ALL)),
}
LN1_CUTS = (0, 96, 192, 256)
LAST_PARTS = ((0, 192), (192, 64))
N_COPIES = 6 + 3 * NCH + 6 + NT + 2 * NF + 1 + (NT - 1) + len(LAST_PARTS)


def _dft_mats():
    ks = np.concatenate([np.arange(0, L, 2), np.arange(1, L, 2)])
    th = 2 * np.pi * (ks + 0.5) / (2 * L)
    j = np.arange(L)
    ang = (th[:, None] * j[None, :]).reshape(L // 8, 1, 8, L)
    Fm = np.concatenate([np.cos(ang), -np.sin(ang)], 1).reshape(2 * L, L)
    Gm = Fm.T / L
    Hm = np.concatenate([-np.sin(ang) - np.cos(ang), np.cos(ang) - np.sin(ang)], 1).reshape(2 * L, L)
    return (np.concatenate([Fm, Hm], 0).astype(jnp.bfloat16), np.ascontiguousarray(Gm).astype(jnp.bfloat16))


def _norm(x):
    m = jnp.sum(x, axis=-1, keepdims=True) * (1.0 / D)
    xc = x - m
    v = jnp.sum(xc * xc, axis=-1, keepdims=True) * (1.0 / D)
    return xc * lax.rsqrt(v + EPS)


def _kernel(q_hbm, k_hbm, v_hbm, s_hbm, w1_hbm, w3_hbm, w2_hbm, wm_hbm, sh_hbm, dd_hbm, c_hbm, f_hbm, g_hbm,
            out_hbm,
            q_v, k_v, v_v, s_v, w1_v, w3_v, w2_v, wm_v, sh_v, dd_v, cc_v, f_v, g_v, one_v,
            f2_v, g2_v, kv_v, u_v, w_v, c_v, y_v, z_v, h_v, n_v, act0_v, act1_v, out_v, mod_v,
            sems):
    f32, bf16 = jnp.float32, jnp.bfloat16
    n_sem = [0]

    def cp(src, dst):
        n_sem[0] += 1
        return pltpu.make_async_copy(src, dst, sems.at[n_sem[0] - 1])

    def wait(copies):
        for c in copies:
            c.wait()

    def rows(j, n):
        return pl.ds(j * n, n)

    small = [cp(a, b) for a, b in (
        (sh_hbm, sh_v), (f_hbm.at[0:16], one_v), (f_hbm, f_v), (dd_hbm, dd_v), (g_hbm, g_v), (c_hbm, cc_v))]
    kvs = [[cp(k_hbm.at[rows(j, CH)], k_v.at[rows(j, CH)]),
            cp(v_hbm.at[rows(j, CH)], v_v.at[rows(j, CH)]),
            cp(s_hbm.at[:, rows(j, CH)], s_v.at[:, rows(j, CH)])] for j in range(NCH)]
    wm = {j: cp(wm_hbm.at[:, rows(j, D)], wm_v.at[:, rows(j, D)]) for j in range(6)}
    qc = [cp(q_hbm.at[rows(t, TM)], q_v.at[rows(t, TM)]) for t in range(NT)]
    w13 = [[cp(w1_hbm.at[:, rows(j, FC)], w1_v.at[:, rows(j, FC)]),
            cp(w3_hbm.at[:, rows(j, FC)], w3_v.at[:, rows(j, FC)])] for j in range(NF)]
    w2c = cp(w2_hbm, w2_v)
    oc = [[cp(out_v.at[rows(t, TM)], out_hbm.at[rows(t, TM)])] for t in range(NT - 1)]
    oc.append([cp(out_v.at[pl.ds(S - TM + r, n)], out_hbm.at[pl.ds(S - TM + r, n)]) for r, n in LAST_PARTS])

    need = [small[:2] + kvs[0][:2], kvs[0][2:] + small[2:4], kvs[1][:2], kvs[1][2:] + small[4:], kvs[2][:2]]
    need += [kvs[j - 1][2:] + kvs[j][:2] for j in range(3, NCH - 1)] + [kvs[NCH - 2][2:] + kvs[NCH - 1][2:]]
    need[-2] += kvs[NCH - 1][:2]
    queue = [c for cs in need for c in cs]
    queue += [wm[2], wm[1], wm[0], qc[0], wm[4], wm[3], qc[1]] + w13[0]
    queue += [c for j in range(1, NF) for c in w13[j]] + [qc[2], wm[5], w2c] + qc[3:]
    for c in queue:
        c.start()

    def gate(r0):
        sh = sh_v[...].astype(f32)
        kb = after(k_v[pl.ds(r0, KR), :], chain.get(0)).astype(f32)
        prev = jnp.zeros((8, D), f32) if r0 == 0 else k_v[pl.ds(r0 - 16, 16), :].astype(f32)[8:]
        kk = jnp.concatenate([prev, kb], axis=0)
        ks = kb * sh[0:1]
        for j in range(1, 4):
            ks = ks + pltpu.roll(kk, j, 0)[8:] * sh[j:j + 1]
        kv = (ks * v_v[pl.ds(r0, KR), :].astype(f32)).astype(bf16)
        kv_v[pl.ds(r0, KR), :] = kv
        link(0, bits(kv))

    def fwd_signal(b):
        u = jnp.dot(f2_v[:2 * L], kv_v[rows(b, L), :], preferred_element_type=f32)
        u_v[b] = u

    def fwd_filter(b):
        w = lax.dot_general(f2_v[2 * L:], s_v[:, rows(b, L)], (((1,), (1,)), ((), ())), preferred_element_type=f32)
        w = w.reshape(NG, 2, 8, D)
        if b == 0:
            dd = dd_v[...].astype(f32).reshape(1, 1, D)
            cq, cr = w[:, 0] - dd, w[:, 1] + dd
            w = jnp.stack([cq, cr], axis=1)
        else:
            p = w_v[(b - 1) % 2].reshape(NG, 2, 8, D)
            H = NG // 2
            cq = jnp.concatenate([w[:H, 0] + p[:H, 1], w[H:, 0] - p[H:, 1]], axis=0)
            cr = jnp.concatenate([w[:H, 1] - p[:H, 0], w[H:, 1] + p[H:, 0]], axis=0)
        c_v[b] = jnp.stack([cq, cr], axis=1).reshape(2 * L, D)
        if b + 1 < NB:
            w_v[b % 2] = w.reshape(2 * L, D)

    def always():
        return bits(one_v[...]) != jnp.uint32(0xFFFFFFFF)

    def bits(x):
        return pltpu.bitcast(x, jnp.uint32)

    def fold(x, n):
        parts = [x[r:r + 8, c:c + 128] for r in range(0, x.shape[0], 8) for c in range(0, x.shape[1], 128)]
        outs = [functools.reduce(jnp.bitwise_or, parts[i::n]) for i in range(n)]
        return outs[0] if n == 1 else jnp.concatenate(outs, axis=1)

    def after(x, dep):
        if dep is None:
            return x
        xi = bits(x)
        reps = (xi.shape[0] // 8, xi.shape[1] // 128)
        if dep.shape != xi.shape:
            dep = jnp.tile(fold(dep, 1), reps)
        return pltpu.bitcast(jnp.where(jnp.tile(always(), reps), xi, dep), x.dtype)

    chain = {}

    def link(key, dep):
        dep = fold(dep, 1)
        chain[key] = dep

    def mac(outs, l, g, parts):
        ls = pl.ds(l * 128, 128)
        acc = {}

        def signal(b, i):
            if i == 0:
                return signal(b, 1) + signal(b, 2)
            return u_v[b, pl.ds(g * 16 + (i - 1) * 8, 8), ls]

        for part in parts:
            for m in range(max(outs) + 1):
                for i in part:
                    cq, cr = pl.ds(g * 16, 8), pl.ds(g * 16 + 8, 8)
                    c = c_v[m, cr, ls] - c_v[m, cq, ls] if i == 0 else c_v[m, cq if i == 1 else cr, ls]
                    if m == 0:
                        c = after(c, chain.get(0))
                    for a in outs:
                        if m <= a:
                            t = c * signal(a - m, i)
                            acc[a, i] = t if m == 0 else acc[a, i] + t
            if part is not parts[-1]:
                link(0, jnp.concatenate([bits(acc[a, i]) for a in outs for i in part], axis=1))
        ys = []
        for a in outs:
            k0 = 0.5 * acc[a, 0]
            y = jnp.concatenate([k0 - acc[a, 2], k0 + acc[a, 1]], axis=0).astype(bf16)
            y_v[pl.ds(a * 2 * L + g * 16, 16), ls] = y
            ys.append(bits(y))
        link(0, jnp.concatenate(ys, axis=1))

    def mod(j):
        cc = cc_v[...].astype(f32)
        sc = jnp.broadcast_to(cc * jax.nn.sigmoid(cc), (16, D)).astype(bf16)
        m = jnp.dot(sc, wm_v[:, rows(j, D)], preferred_element_type=f32)[:8]
        if j in (1, 4):
            m = 1 + m
        if j in (0, 1):
            m = m * mod_v[2]
        mod_v[j] = m

    def ln(r0, key):
        rs = pl.ds(r0, LNR)
        sa, ca, sb, cb = [jnp.tile(mod_v[j], (LNR // 8, 1)) for j in (0, 1, 3, 4)]
        x = after(q_v[rs, :], chain.get(key)).astype(f32)
        x1 = x + (_norm(x) * ca + sa) * z_v[rs, :]
        z_v[rs, :] = x1
        h = (_norm(x1) * cb + sb).astype(bf16)
        h_v[rs, :] = h
        link(key, bits(h))

    def ln_first_a(r0):
        rs = pl.ds(r0, LNR)
        sa, ca = [jnp.tile(mod_v[j], (LNR // 8, 1)) for j in range(2)]
        x = q_v[rs, :].astype(f32)
        x1 = x + (_norm(x) * ca + sa) * z_v[rs, :]
        z_v[rs, :] = x1
        n_v[rs, :] = _norm(x1)

    def ln_first_b(r0):
        rs = pl.ds(r0, LNR)
        sb, cb = [jnp.tile(mod_v[j], (LNR // 8, 1)) for j in (3, 4)]
        h_v[rs, :] = (n_v[rs, :] * cb + sb).astype(bf16)

    def up(t, j):
        h = h_v[rows(t, TM), :]
        w1, w3 = w1_v[:, rows(j, FC)], w3_v[:, rows(j, FC)]
        g = 0.5 * jnp.dot(h, w1, preferred_element_type=f32)
        u = jnp.dot(h, w3, preferred_element_type=f32)
        (act0_v, act1_v)[t % 2][:, rows(j, FC)] = ((g * jnp.tanh(g) + g) * u).astype(bf16)

    def down(t):
        w2 = w2_v[...]
        for c, (r, n) in zip(oc[t], LAST_PARTS if t == NT - 1 else ((0, TM),)):
            o = jnp.dot((act0_v, act1_v)[t % 2][pl.ds(r, n), :], w2, preferred_element_type=f32)
            rs = pl.ds(t * TM + r, n)
            out_v[rs, :] = (z_v[rs, :] + jnp.tile(mod_v[5], (n // 8, 1)) * o).astype(bf16)
            c.start()

    def run(tasks):
        for kind, j, *rest in tasks:
            if kind == "gate":
                for r0 in range(j * CH, (j + 1) * CH, KR):
                    gate(r0)
            elif kind == "fw":
                fwd_filter(2 * j)
                fwd_filter(2 * j + 1)
            elif kind == "fu":
                fwd_signal(2 * j)
                fwd_signal(2 * j + 1)
            elif kind == "inv":
                ls = pl.ds(rest[0][0] * 128, len(rest[0]) * 128)
                for b in (2 * j, 2 * j + 1):
                    z_v[rows(b, L), ls] = jnp.dot(g2_v[...], y_v[rows(b, 2 * L), ls], preferred_element_type=f32)
            else:
                parts = ((0,), (1,), (2,)) if rest[1:] else ((0, 1, 2),)
                for l in rest[0]:
                    for g in range(NG):
                        mac((2 * j, 2 * j + 1), l, g, parts)

    for j, tasks in enumerate(PROLOGUE):
        wait(need[j])
        if j == 1:
            f2_v[...] = f_v[...]
        if j == 3:
            g2_v[...] = g_v[...]
        chain.clear()
        run(tasks)

    wait((wm[2], wm[1], wm[0], qc[0], wm[4], wm[3]))
    chain.clear()
    for j in (2, 1, 0):
        mod(j)
    for r0 in range(0, TM, LNR):
        ln_first_a(r0)
    for j in (4, 3):
        mod(j)
    for r0 in range(0, TM, LNR):
        ln_first_b(r0)

    for j in range(3):
        wait(w13[j] + ([qc[1]] if j == 0 else []))
        chain.clear()
        for i, r0 in enumerate(range(LN1_CUTS[j], LN1_CUTS[j + 1], LNR)):
            ln(TM + r0, "ln%d" % (i % 3))
        up(0, j)
    for j in range(3):
        up(1, j)
    wait(w13[3] + w13[4] + w13[5] + [qc[2]])
    chain.clear()
    for r0 in range(0, TM // 2, LNR):
        ln(2 * TM + r0, "ln")
    for j in range(3, NF):
        up(0, j)
        up(1, j)
    wait([wm[5], w2c, qc[3], qc[4]])
    mod(5)
    chain.clear()
    for r0 in range(TM // 2, TM, LNR):
        ln(2 * TM + r0, "ln")
    down(0)
    down(1)

    def late(*pos):
        if pos in LATE:
            chain.pop(0, None)
            run(LATE[pos])

    for t in range(2, NT):
        if t == 4:
            wait(qc[5:])
            chain.clear()
        for j in range(NF):
            late(t, j)
            if j == 0 and t + 1 < NT:
                for r0 in range((t + 1) * TM, (t + 2) * TM, LNR):
                    ln(r0, "ln")
            up(t, j)
        late(t, NF)
        down(t)
    wait([c for cs in oc for c in cs])


def pallas_adaLN_cond__ssm_conv_h3__glu_gated_swiglu__prompt_kernel(
        A_q, A_k, A_v, A_shift_k, A_ssm_k, A_ssm_D, B_x, B_w1, B_w3, B_w2, c, w_mod):
    Fm, Gm = _dft_mats()
    f32, bf16 = jnp.float32, jnp.bfloat16
    anyspec = pl.BlockSpec(memory_space=pl.ANY)
    V = pltpu.VMEM
    dma = pltpu.SemaphoreType.DMA
    out = pl.pallas_call(
        _kernel,
        in_specs=[anyspec] * 13,
        out_specs=anyspec,
        out_shape=jax.ShapeDtypeStruct((S, D), bf16),
        scratch_shapes=[
            V((S, D), bf16), V((S, D), bf16), V((S, D), bf16), V((D, S), bf16),
            V((D, FF), bf16), V((D, FF), bf16), V((FF, D), bf16), V((D, 6 * D), bf16),
            V((4, D), bf16), V((D,), bf16), V((1, D), bf16), V((4 * L, L), bf16), V((L, 2 * L), bf16), V((16, L), bf16),
            V((4 * L, L), bf16), V((L, 2 * L), bf16),
            V((S, D), bf16), V((NB, 2 * L, D), f32), V((2, 2 * L, D), f32), V((NB, 2 * L, D), f32), V((NB * 2 * L, D), bf16),
            V((S, D), f32), V((S, D), bf16), V((TM, D), f32), V((TM, FF), bf16), V((TM, FF), bf16), V((S, D), bf16), V((6, 8, D), f32),
            dma((N_COPIES,)),
        ],
        compiler_params=pltpu.CompilerParams(vmem_limit_bytes=110 * 1024 * 1024),
    )(A_q.reshape(S, D), A_k.reshape(S, D), A_v.reshape(S, D), A_ssm_k, B_w1, B_w3, B_w2, w_mod,
      A_shift_k.T, A_ssm_D, c, Fm, Gm)
    return out.reshape(1, S, D)
```
